```python
import jax
import jax.numpy as jnp

def _softmax(x, axis=-1):
    return jax.nn.softmax(x, axis=axis)
def _gelu(x):
    return jax.nn.gelu(x, approximate=True)
def _silu(x):
    return jax.nn.silu(x)
def _sigmoid(x):
    return jax.nn.sigmoid(x)
def _layernorm(x, axis=-1, eps=1e-5):
    m = jnp.mean(x, axis=axis, keepdims=True)
    v = jnp.var(x, axis=axis, keepdims=True)
    return (x - m) / jnp.sqrt(v + eps)
def _scatter_add(tgt, idx, src, axis=0):
    return tgt.at[idx].add(src)
def _segment_sum(src, seg, n):
    return jax.ops.segment_sum(src, seg, n)
class _Rng:
    def __init__(self, key):
        self._k = key
    def _next(self):
        self._k, sub = jax.random.split(self._k)
        return sub
    def normal(self, shape):
        return jax.random.normal(self._next(), shape, dtype=jnp.bfloat16)
    def randint(self, lo, hi, shape):
        return jax.random.randint(self._next(), shape, lo, hi, dtype=jnp.int32)
    def uniform(self, shape, lo=0.0, hi=1.0):
        return jax.random.uniform(self._next(), shape, jnp.bfloat16, lo, hi)
    def permutation(self, n):
        return jax.random.permutation(self._next(), n)


kernel_name = 'standalone__fused_io_aware_attn__prompt'

def setup_inputs():
    _rng = _Rng(jax.random.key(int.from_bytes(__import__("os").urandom(4), "little")))
    _w = (lambda a: (lambda t: t.astype(jnp.bfloat16) if jnp.issubdtype(t.dtype, jnp.floating) else t)(jnp.asarray(a)))
    B, H, S = 2, 32, 2048
    Dh = max(1, 1024 // 32)
    return {
        "q": _w((lambda *s: _rng.normal(s) * 0.05)(B, H, S, Dh)),
        "k": _w((lambda *s: _rng.normal(s) * 0.05)(B, H, S, Dh)),
        "v": _w((lambda *s: _rng.normal(s) * 0.05)(B, H, S, Dh)),
    }

def reference(q, k, v):
    scale = q.shape[-1] ** -0.5
    s = jnp.einsum('bhqd,bhkd->bhqk', q, k) * scale
    p = _softmax(s, axis=-1)
    return jnp.einsum('bhqk,bhkd->bhqd', p, v)
```

```python
import functools
import math

import jax
import jax.numpy as jnp
import jax.experimental.pallas as pl
import jax.experimental.pallas.tpu as pltpu

_TQ = 128
_G = 4
_LAG = 2
_EDEP = 2


def _attn_kernel(q_ref, k_ref, v_ref, o_ref, kk_ref, vv_ref, qq_ref):
    D, S = q_ref.shape[2], q_ref.shape[3]
    TQ, G = _TQ, _G
    CK = 128 * G
    c = (D ** -0.5) * math.log2(math.e)
    kk_ref[...] = pltpu.bitcast(k_ref[0, 0].T, jnp.uint32)
    vv_ref[...] = pltpu.bitcast(v_ref[0, 0], jnp.uint32)
    qq_ref[...] = pltpu.bitcast(
        (q_ref[0, 0].astype(jnp.float32) * c).astype(jnp.bfloat16), jnp.uint32)
    nt = S // TQ
    nc = S // CK
    never = jnp.full((8, TQ), pl.program_id(0) >> 20, jnp.int32) != 0
    N = nt * nc
    s_vals, m_hist, m_fin = {}, {}, {}
    for n in range(N + nc + _LAG):
        if n < N:
            i, j = divmod(n, nc)
            qw = pltpu.bitcast(qq_ref[:, i * TQ:(i + 1) * TQ], jnp.bfloat16)
            ss = []
            for g in range(G):
                r0 = (j * CK + g * 128) // 2
                kg = pltpu.bitcast(kk_ref[r0:r0 + 64, :], jnp.bfloat16)
                ss.append(jnp.dot(kg, qw, preferred_element_type=jnp.float32))
            s_vals[n] = ss
            ms = []
            for g in range(G):
                mm = None if j == 0 else m_hist[n - 1][g]
                for r in range(16):
                    x = ss[g][r * 8:(r + 1) * 8]
                    mm = x if mm is None else jnp.maximum(mm, x)
                ms.append(mm)
            m_hist[n] = ms
            if j == nc - 1:
                mm = functools.reduce(jnp.maximum, ms)
                m_fin[i] = jnp.broadcast_to(
                    jnp.max(mm, axis=0, keepdims=True), (8, TQ))
        nb = n - nc - _LAG
        if nb >= 0:
            i, j = divmod(nb, nc)
            ss = s_vals.pop(nb)
            if j == 0:
                l_run = [None] * G
            ps = []
            for g in range(G):
                m8 = m_fin[i]
                if n - _EDEP < N:
                    m8 = jnp.where(never, m_hist[n - _EDEP][g], m8)
                rows = [None] * 16
                for r in reversed(range(16)):
                    p = jnp.exp2(ss[g][r * 8:(r + 1) * 8] - m8)
                    l_run[g] = p if l_run[g] is None else l_run[g] + p
                    if r == 0:
                        p = jnp.where(never, l_run[g], p)
                    rows[r] = p
                ps.append(jnp.concatenate(rows, axis=0).astype(jnp.bfloat16))
            for g in range(G):
                c0 = j * CK + g * 128
                vg = pltpu.bitcast(vv_ref[:, c0:c0 + 128], jnp.bfloat16)
                pv = jnp.dot(vg, ps[g], preferred_element_type=jnp.float32)
                acc = pv if (j == 0 and g == 0) else acc + pv
            if j == nc - 1:
                l = jnp.sum(functools.reduce(jnp.add, l_run), axis=0, keepdims=True)
                o_ref[0, 0, :, i * TQ:(i + 1) * TQ] = (
                    acc * (1.0 / l)).astype(o_ref.dtype)


@jax.jit
def pallas_standalone__fused_io_aware_attn__prompt_kernel(
    q: jax.Array,
    k: jax.Array,
    v: jax.Array,
):
    B, H, S, D = q.shape
    qt, kt, vt = (jnp.swapaxes(x, -1, -2) for x in (q, k, v))
    spec = pl.BlockSpec((1, 1, D, S), lambda b, h: (b, h, 0, 0))
    ot = pl.pallas_call(
        _attn_kernel,
        grid=(B, H),
        in_specs=[spec, spec, spec],
        out_specs=spec,
        out_shape=jax.ShapeDtypeStruct((B, H, D, S), q.dtype),
        scratch_shapes=[
            pltpu.VMEM((S // 2, D), jnp.uint32),
            pltpu.VMEM((D // 2, S), jnp.uint32),
            pltpu.VMEM((D // 2, S), jnp.uint32),
        ],
        compiler_params=pltpu.CompilerParams(
            dimension_semantics=("parallel", "parallel"),
            vmem_limit_bytes=64 << 20),
    )(qt, kt, vt)
    return jnp.swapaxes(ot, -1, -2)
```

```python
import functools
import math

import jax
import jax.numpy as jnp
from jax import lax
import jax.experimental.pallas as pl
import jax.experimental.pallas.tpu as pltpu

f32, bf16, u32, i32 = jnp.float32, jnp.bfloat16, jnp.uint32, jnp.int32

_TQ = 128
_KD = 80
_ORDER = (6, 4, 2, 0, 7, 5, 3, 1)
_T_MAX = 64.0
_HPS = 7
_G = 2
_LAG = 3
_NL = 4
_P0, _PEND = 2, 3


def _scale(d):
    return (d ** -0.5) * math.log2(math.e)


def _sumsq(x):
    y = x * x
    return (y[0:8] + y[8:16]) + (y[16:24] + y[24:32])


def _prep_items(h, slot, refs, tie, after):
    q_ref, k_ref, v_ref, _, kk_ref, vv_ref, mm_ref, flag_ref = refs
    D, S = q_ref.shape[1], q_ref.shape[2]
    H2 = S // 2
    c = _scale(D)
    st = {}

    def upd(key, n2):
        n2 = after(n2)
        st[key] = jnp.maximum(st[key], n2) if key in st else n2
        tie(st[key])

    def q_item(i):
        upd('q', _sumsq(q_ref[h, :, i * _TQ:(i + 1) * _TQ].astype(f32)))

    def k_item(t):
        ka = k_ref[h, :, t * 128:(t + 1) * 128].astype(f32)
        kb = k_ref[h, :, H2 + t * 128:H2 + (t + 1) * 128].astype(f32)
        upd('k', jnp.maximum(_sumsq(ka), _sumsq(kb)))
        xt = jnp.concatenate(
            [ka * c, jnp.ones((16, 128), f32), kb * (c * 2.0 ** -13),
             jnp.zeros((48, 128), f32)], axis=0).astype(bf16)
        kt = pltpu.bitcast(xt.T, u32)
        kk_ref[slot, t * 64:(t + 1) * 64, :] = jnp.concatenate(
            [kt[8 * w:8 * w + 8] for w in _ORDER], axis=0)
        tie(pltpu.bitcast(kt[56:64], f32))

    def v_item(t):
        lane = lax.broadcasted_iota(i32, (16, 128), 1)
        sel = (lane & 16) == 0
        va = pltpu.bitcast(v_ref[h, :, t * 128:(t + 1) * 128], u32)
        vb = pltpu.bitcast(v_ref[h, :, H2 + t * 128:H2 + (t + 1) * 128], f32)
        vb = pltpu.bitcast(
            jnp.concatenate([after(vb[0:8]), after(vb[8:16])], axis=0), u32)
        v1 = jnp.where(sel, va, pltpu.roll(vb, 16, 1))
        v2 = jnp.where(sel, pltpu.roll(vb, 112, 1), va)
        vv_ref[slot, :, t * 128:(t + 1) * 128] = v1
        vv_ref[slot, :, H2 + t * 128:H2 + (t + 1) * 128] = v2
        for z in (v2[8:16], v2[0:8], v1[8:16], v1[0:8]):
            tie(pltpu.bitcast(z, f32))

    def fin():
        def top(x):
            x = jnp.sum(x, axis=0, keepdims=True)
            return jnp.max(x, axis=1, keepdims=True) + 2.0 ** -120
        b2 = jnp.broadcast_to(top(st['q']) * top(st['k']) * (1.04 * c * c), (8, 128))
        safe = jnp.min(jnp.where(b2 < _T_MAX * _T_MAX, 1, 0))
        flag_ref[slot] = safe * flag_ref[_HPS]
        b2 = jnp.minimum(jnp.maximum(b2, 2.0 ** -40), _T_MAX * _T_MAX)
        e = (pltpu.bitcast(b2, i32) >> 23) - 127
        p2 = pltpu.bitcast(((e >> 1) + 128) << 23, f32)
        cm = p2 * 3072.0
        row = lax.broadcasted_iota(i32, (8, 128), 0)
        cz = jnp.where(row == 0, cm, jnp.where(row == 4, -cm, 0.0))
        crow = pltpu.bitcast(pltpu.bitcast(cz, u32) >> 16, f32)
        mm_ref[slot, 0] = cm
        mm_ref[slot, 1] = crow
        tie(crow)

    items = []
    for t in range(S // 256):
        items += [functools.partial(k_item, t), functools.partial(q_item, 2 * t),
                  functools.partial(v_item, t), functools.partial(q_item, 2 * t + 1)]
    return items, fin


def _prep_head(h, slot, refs):
    items, fin = _prep_items(h, slot, refs, lambda x: None, lambda x: x)
    for it in items + [fin]:
        it()


def _accumulation_check():
    row = lax.broadcasted_iota(i32, (_KD, 128), 0)
    w = jnp.where(row < 32, 0.0107421875,
                  jnp.where(row == 32, 6291456.0,
                            jnp.where(row == 40, -6291456.0,
                                      jnp.where(row >= 48, 2.0 ** -9, 0.0))))
    r = jnp.dot(jnp.ones((128, _KD), bf16), w.astype(bf16), preferred_element_type=f32)
    return jnp.min(jnp.where(r == 0.5625, 1, 0))


def _packed_heads(h0, slots, refs, never, head_done):
    q_ref, _, v_ref, o_ref, kk_ref, vv_ref, mm_ref, _ = refs
    S = v_ref.shape[2]
    H2 = S // 2
    G, TQ = _G, _TQ
    nc = H2 // (128 * G)
    NH = (S // TQ) * nc
    N = NH * len(slots)
    F = 4 // G
    xs, ties, sched, now = {}, [], {}, {}

    def after(x):
        return jnp.where(never, now['v'], x)

    for a in range(len(slots)):
        if a + 1 < len(slots):
            hn, sn = h0 + a + 1, slots[a + 1]
        else:
            hn, sn = jnp.minimum(h0 + a + 1, q_ref.shape[0] - 1), 0
        items, fin = _prep_items(hn, sn, refs, ties.append, after)
        ns = NH - (_P0 + _PEND + 2) * F
        for b, it in enumerate(items):
            sched.setdefault(a * NH + _P0 * F + b * ns // len(items), []).append(it)
        sched.setdefault(a * NH + NH - _PEND * F - 1, []).append(fin)
        sched.setdefault(min(N - 1, a * NH + NH + 3), []).append(
            functools.partial(head_done, a))

    for n in range(N + _LAG):
        if n < N:
            a, rem = divmod(n, NH)
            i, j = divmod(rem, nc)
            sl = slots[a]
            qu = pltpu.bitcast(q_ref[h0 + a, :, i * TQ:(i + 1) * TQ], u32)
            qw = pltpu.bitcast(jnp.concatenate(
                [qu, pltpu.bitcast(mm_ref[sl, 1], u32), qu], axis=0), bf16)
            xs[n] = []
            for g in range(G):
                r0 = (j * G + g) * 64
                kg = pltpu.bitcast(kk_ref[sl, r0:r0 + 64, :], bf16)[:, :_KD]
                xs[n].append(jnp.dot(kg, qw, preferred_element_type=f32))
        nb = n - _LAG
        if nb < 0:
            continue
        a, rem = divmod(nb, NH)
        i, j = divmod(rem, nc)
        sl = slots[a]
        if rem == 0:
            cm = mm_ref[sl, 0][None]
        if j == 0:
            l_run = [None] * _NL
        tiles = []
        for g, x in enumerate(xs.pop(nb)):
            lg = (j * G + g) % _NL
            x = x.reshape(16, 8, 128)
            hi = (x + cm) - cm
            ph = jnp.exp2(hi)
            plo = jnp.exp2((x - hi) * 8192.0)
            t = ph + plo
            s1 = jnp.sum(t[0:8], axis=0)
            l1 = s1 if l_run[lg] is None else l_run[lg] + s1
            l_run[lg] = l1 + jnp.sum(t[8:16], axis=0)
            t1 = jnp.concatenate(
                [ph[6:7], jnp.where(never, l1, ph[7])[None], plo[6:8], ph[4:6],
                 plo[4:6], ph[2:4], plo[2:4], ph[0:2], plo[0:2]], axis=0)
            t2 = jnp.concatenate(
                [plo[14:15], jnp.where(never, l_run[lg], plo[15])[None], ph[14:16],
                 plo[12:14], ph[12:14], plo[10:12], ph[10:12], plo[8:10], ph[8:10]],
                axis=0)
            tiles.append((t1.reshape(128, 128).astype(bf16),
                          t2.reshape(128, 128).astype(bf16)))
        for half in range(2):
            for g in range(G):
                c0 = half * H2 + (j * G + g) * 128
                vg = pltpu.bitcast(vv_ref[sl, :, c0:c0 + 128], bf16)
                pv = jnp.dot(vg, tiles[g][half], preferred_element_type=f32)
                if j == 0 and g == 0 and half == 0:
                    acc = pv
                    continue
                if ties:
                    acc = jnp.concatenate(
                        [acc[0:24], jnp.where(never, ties.pop(0), acc[24:32])], axis=0)
                acc = acc + pv
        if j == nc - 1:
            l = jnp.sum(functools.reduce(jnp.add, l_run), axis=0, keepdims=True)
            o_ref[h0 + a, :, i * TQ:(i + 1) * TQ] = (acc * (1.0 / l)).astype(o_ref.dtype)
        now['v'] = now.get('w')
        now['w'] = l1
        for it in sched.pop(nb, []):
            it()
    assert not sched and not ties


def _exact_head(h, refs):
    q_ref, k_ref, v_ref, o_ref = refs[:4]
    D, S = v_ref.shape[1], v_ref.shape[2]
    TS = 512

    def body(it, carry):
        c0 = pl.multiple_of(it * TS, TS)
        qw = (q_ref[h, :, pl.ds(c0, TS)].astype(f32) * _scale(D)).astype(bf16)
        s = lax.dot_general(k_ref[h], qw, (((0,), (0,)), ((), ())),
                            preferred_element_type=f32)
        p = jnp.exp2(s - jnp.max(s, axis=0, keepdims=True))
        l = jnp.sum(p, axis=0, keepdims=True)
        acc = jnp.dot(v_ref[h], p.astype(bf16), preferred_element_type=f32)
        o_ref[h, :, pl.ds(c0, TS)] = (acc * (1.0 / l)).astype(o_ref.dtype)
        return carry

    lax.fori_loop(0, S // TS, body, 0)


def _kernel(q_hbm, k_hbm, v_hbm, o_hbm, q_ref, k_ref, v_ref, o_ref,
            kk_ref, vv_ref, mm_ref, flag_ref, redo_ref, sem_in, sem_out):
    HPS = _HPS
    t = pl.program_id(0)
    n_heads = q_ref.shape[0]
    n_blocks = (n_heads - 1) // HPS
    never = jnp.full((8, _TQ), t >> 20, i32) != 0
    refs = (q_ref, k_ref, v_ref, o_ref, kk_ref, vv_ref, mm_ref, flag_ref)
    ins = ((k_hbm, k_ref), (q_hbm, q_ref), (v_hbm, v_ref))

    def cp_in(h, n, s):
        return [pltpu.make_async_copy(hbm.at[pl.ds(h, n)], buf.at[pl.ds(h, n)],
                                      sem_in.at[3 * s + a])
                for a, (hbm, buf) in enumerate(ins)]

    def block_in(b, op):
        h = 2 + (b - 1) * HPS

        @pl.when(b < n_blocks)
        def _():
            for cp in cp_in(h, HPS, b % 2):
                op(cp)

        @pl.when(b == n_blocks)
        def _():
            for cp in cp_in(h, HPS - 1, b % 2):
                op(cp)

    def cp_out(h):
        return pltpu.make_async_copy(o_ref.at[h], o_hbm.at[h], sem_out.at[0])

    def run_block(h0, slots):
        ok0 = flag_ref[slots[0]]
        redo_ref[HPS] = ok0

        def head_done(a):
            ok = ok0 if a == 0 else flag_ref[slots[a]]
            redo_ref[a] = 1 - ok

            @pl.when(ok != 0)
            def _():
                cp_out(h0 + a).start()

        @pl.when(ok0 != 0)
        def _():
            _packed_heads(h0, slots, refs, never, head_done)

    @pl.when(t == 0)
    def _():
        for cp in cp_in(0, 1, 0) + cp_in(1, 1, 2):
            cp.start()
        flag_ref[HPS] = _accumulation_check()
        for cp in cp_in(0, 1, 0):
            cp.wait()
        block_in(1, lambda cp: cp.start())
        _prep_head(0, HPS - 1, refs)
        for cp in cp_in(1, 1, 2):
            cp.wait()
        run_block(0, [HPS - 1])

    @pl.when(t > 0)
    def _():
        block_in(t + 1, lambda cp: cp.start())
        block_in(t, lambda cp: cp.wait())
        run_block(1 + (t - 1) * HPS, list(range(HPS)))

    h0 = jnp.where(t == 0, 0, 1 + (t - 1) * HPS)
    n = jnp.where(t == 0, 1, HPS)

    @pl.when(redo_ref[HPS] == 0)
    def _():
        for a in range(HPS):
            redo_ref[a] = 1
        _prep_head(jnp.minimum(h0 + n, n_heads - 1), 0, refs)

    def fix(a, carry):
        @pl.when(redo_ref[a] != 0)
        def _():
            _exact_head(h0 + a, refs)
            cp_out(h0 + a).start()
        return carry

    lax.fori_loop(0, n, fix, 0)

    @pl.when(t == n_blocks)
    def _():
        pltpu.make_async_copy(o_ref, o_hbm, sem_out.at[0]).wait()


@jax.jit
def pallas_standalone__fused_io_aware_attn__prompt_kernel(
    q: jax.Array,
    k: jax.Array,
    v: jax.Array,
):
    B, H, S, D = q.shape
    n_heads = B * H
    assert D == 32 and S % 512 == 0 and (n_heads - 1) % _HPS == 0
    qt, kt, vt = (jnp.swapaxes(x, -1, -2).reshape(n_heads, D, S) for x in (q, k, v))
    hbm = pl.BlockSpec(memory_space=pl.ANY)
    resident = pltpu.VMEM((n_heads, D, S), q.dtype)
    ot = pl.pallas_call(
        _kernel,
        grid=((n_heads - 1) // _HPS + 1,),
        in_specs=[hbm] * 3,
        out_specs=hbm,
        out_shape=jax.ShapeDtypeStruct((n_heads, D, S), q.dtype),
        scratch_shapes=[
            resident, resident, resident, resident,
            pltpu.VMEM((_HPS, S // 4, 128), u32),
            pltpu.VMEM((_HPS, D // 2, S), u32),
            pltpu.VMEM((_HPS, 2, 8, 128), f32),
            pltpu.SMEM((_HPS + 1,), i32),
            pltpu.SMEM((_HPS + 1,), i32),
            pltpu.SemaphoreType.DMA((9,)),
            pltpu.SemaphoreType.DMA((1,)),
        ],
        compiler_params=pltpu.CompilerParams(
            dimension_semantics=("arbitrary",),
            vmem_limit_bytes=96 << 20,
            disable_bounds_checks=True),
    )(qt, kt, vt)
    return jnp.swapaxes(ot.reshape(B, H, D, S), -1, -2)
```

```python
import functools
import math

import jax
import jax.numpy as jnp
from jax import lax
import jax.experimental.pallas as pl
import jax.experimental.pallas.tpu as pltpu

f32, bf16, u32, i32 = jnp.float32, jnp.bfloat16, jnp.uint32, jnp.int32

_TQ = 128
_KD = 80
_ORDER = (6, 4, 2, 0, 7, 5, 3, 1)
_T_MAX = 64.0
_HPS = 7
_NL = 4
_TS = 512
_OSPLIT = 14
_PREFIX = ("QQ", "QQ", "QQPPP", "QQPPP")
_TAILP = 6
_P0, _PEND, _GAP, _AFT, _TDLY = 16, 32, 3, 3, 4


def _scale(d):
    return (d ** -0.5) * math.log2(math.e)


def _sumsq(x):
    y = x * x
    return (y[0:8] + y[8:16]) + (y[16:24] + y[24:32])


def _prep_items(h, slot, refs, tie, after):
    q_ref, k_ref, v_ref, _, kk_ref, vv_ref, mm_ref, safe_ref = refs
    D, S = q_ref.shape[1], q_ref.shape[2]
    H2 = S // 2
    c = _scale(D)
    st = {}

    def norm_item(key, ref, i):
        n2 = after(_sumsq(ref[h, :, i * 128:(i + 1) * 128].astype(f32)))
        st[key] = jnp.maximum(st[key], n2) if key in st else n2
        tie(st[key])

    def bound_item():
        def top(x):
            x = jnp.sum(x, axis=0, keepdims=True)
            return jnp.max(x, axis=1, keepdims=True) + 2.0 ** -120
        b2 = jnp.broadcast_to(top(st['q']) * top(st['k']) * (1.04 * c * c), (8, 128))
        safe_ref[h] = jnp.where(b2 < _T_MAX * _T_MAX, 1.0, 0.0)
        b2 = jnp.minimum(jnp.maximum(b2, 2.0 ** -40), _T_MAX * _T_MAX)
        e = (pltpu.bitcast(b2, i32) >> 23) - 127
        p2 = pltpu.bitcast(((e >> 1) + 128) << 23, f32)
        cm = p2 * 3072.0
        row = lax.broadcasted_iota(i32, (8, 128), 0)
        cz = jnp.where(row == 0, cm, jnp.where(row == 4, -cm, 0.0))
        crow = pltpu.bitcast(pltpu.bitcast(cz, u32) >> 16, f32)
        mm_ref[slot, 0] = cm
        mm_ref[slot, 1] = crow
        tie(crow)

    def k_item(t):
        ka = k_ref[h, :, t * 128:(t + 1) * 128].astype(f32)
        kb = k_ref[h, :, H2 + t * 128:H2 + (t + 1) * 128].astype(f32)
        xt = jnp.concatenate(
            [ka * c, jnp.ones((16, 128), f32), kb * (c * 2.0 ** -13),
             jnp.zeros((48, 128), f32)], axis=0).astype(bf16)
        kt = pltpu.bitcast(xt.T, u32)
        kk_ref[slot, t * 64:(t + 1) * 64, :] = jnp.concatenate(
            [kt[8 * w:8 * w + 8] for w in _ORDER], axis=0)
        tie(pltpu.bitcast(kt[56:64], f32))

    def v_item(t):
        lane = lax.broadcasted_iota(i32, (16, 128), 1)
        sel = (lane & 16) == 0
        va = pltpu.bitcast(v_ref[h, :, t * 128:(t + 1) * 128], u32)
        vb = pltpu.bitcast(v_ref[h, :, H2 + t * 128:H2 + (t + 1) * 128], f32)
        vb = pltpu.bitcast(
            jnp.concatenate([after(vb[0:8]), after(vb[8:16])], axis=0), u32)
        v1 = jnp.where(sel, va, pltpu.roll(vb, 16, 1))
        v2 = jnp.where(sel, pltpu.roll(vb, 112, 1), va)
        vv_ref[slot, :, t * 128:(t + 1) * 128] = v1
        vv_ref[slot, :, H2 + t * 128:H2 + (t + 1) * 128] = v2
        for z in (v2[8:16], v2[0:8], v1[8:16], v1[0:8]):
            tie(pltpu.bitcast(z, f32))

    part = functools.partial
    gap = [None] * _GAP
    items = []
    for i in range(S // 128):
        items += [part(norm_item, 'q', q_ref, i), part(norm_item, 'k', k_ref, i)]
    items += gap + [bound_item] + gap
    for t in range(0, S // 256, 2):
        items += [part(k_item, t), part(k_item, t + 1)] + gap
    for t in range(S // 256):
        items += [part(v_item, t), None]
    return items


def _prep_head(h, slot, refs):
    for it in _prep_items(h, slot, refs, lambda x: None, lambda x: x):
        if it is not None:
            it()


def _accumulation_probe():
    row = lax.broadcasted_iota(i32, (_KD, 128), 0)
    w = jnp.where(row < 32, 0.0107421875,
                  jnp.where(row == 32, 6291456.0,
                            jnp.where(row == 40, -6291456.0,
                                      jnp.where(row >= 48, 2.0 ** -9, 0.0))))
    return jnp.dot(jnp.ones((128, _KD), bf16), w.astype(bf16),
                   preferred_element_type=f32).reshape(16, 8, 128)


def _mxu_order(nu):
    qs, ps = [], []
    for m, pre in enumerate(_PREFIX):
        nq, npv = nu // 4 - pre.count('Q'), nu // 2 - pre.count('P')
        short = max(0, _TAILP - (npv - 2 * (nq - 1)))
        seq = pre + 'QPP' * (nq - 1 - short) + 'QP' * short + 'Q'
        seq += 'P' * (nu // 2 - seq.count('P'))
        tm = 0
        for ch in seq:
            (qs if ch == 'Q' else ps).append((tm, m))
            tm += 128 if ch == 'Q' else 32
    qs.sort()
    ps.sort()
    ops = {pos: ('Q', u, 0) for u, pos in enumerate(qs)}
    ready = sorted((tm + 64 * (half + 1), u, half)
                   for u, (tm, _) in enumerate(qs) for half in range(2))
    for pos, (_, u, half) in zip(ps, ready):
        ops[pos] = ('P', u, half)
    return [ops[pos] for pos in sorted(ops)]


def _packed_heads(h0, slots, refs, never, events):
    q_ref, _, v_ref, o_ref, kk_ref, vv_ref, mm_ref, _ = refs
    S = v_ref.shape[2]
    H2 = S // 2
    TQ = _TQ
    UT = H2 // 128
    UH = (S // TQ) * UT
    PH = 2 * UH
    xs, tiles, ties, sched, hist = {}, {}, [], {}, []
    qws, cms, lsum, accs, nacc = {}, {}, {}, {}, {}

    def tie(v):
        ties.append((len(hist) + _TDLY, v))

    def after(x):
        return jnp.where(never, hist[-_AFT], x)

    for a in range(len(slots)):
        if a + 1 < len(slots):
            hn, sn = h0 + a + 1, slots[a + 1]
        else:
            hn, sn = jnp.minimum(h0 + a + 1, q_ref.shape[0] - 1), 0
        items = _prep_items(hn, sn, refs, tie, after)
        for b, it in enumerate(items):
            if it is not None:
                at = a * PH + _P0 + b * (PH - _P0 - _PEND) // len(items)
                sched.setdefault(at, []).append(it)

    def softmax_stage(u):
        cm = cms[u // UH]
        l_run = lsum.setdefault(u // UT, [None] * _NL)
        lg = u % _NL
        xu = xs.pop(u)
        for half in range(2):
            x = xu[half * 64:(half + 1) * 64].reshape(8, 8, 128)
            hi = (x + cm) - cm
            ph = jnp.exp2(hi)
            plo = jnp.exp2((x - hi) * 8192.0)
            s1 = jnp.sum(ph + plo, axis=0)
            l1 = l_run[lg] = s1 if l_run[lg] is None else l_run[lg] + s1
            pa, pb = (ph, plo) if half == 0 else (plo, ph)
            pt = jnp.concatenate(
                [pa[6:7], jnp.where(never, l1, pa[7])[None], pb[6:8], pa[4:6],
                 pb[4:6], pa[2:4], pb[2:4], pa[0:2], pb[0:2]], axis=0)
            tiles[(u, half)] = (pt.reshape(128, 128).astype(bf16), l1)

    n_soft = n_out = 0
    for kind, u, half in _mxu_order(UH * len(slots)):
        a, rem = divmod(u, UH)
        i, j = divmod(rem, UT)
        sl = slots[a]
        ti = u // UT
        if kind == 'Q':
            if u // 2 not in qws:
                qu = pltpu.bitcast(q_ref[h0 + a, :, i * TQ:(i + 1) * TQ], u32)
                qws[u // 2] = pltpu.bitcast(jnp.concatenate(
                    [qu, pltpu.bitcast(mm_ref[sl, 1], u32), qu], axis=0), bf16)
            kg = pltpu.bitcast(kk_ref[sl, j * 64:(j + 1) * 64, :], bf16)[:, :_KD]
            xs[u] = jnp.dot(kg, qws[u // 2], preferred_element_type=f32)
            if a not in cms:
                cms[a] = mm_ref[sl, 0][None]
            if u == UT - 1:
                for fn in events.pop(0, []):
                    fn()
            continue
        while n_soft <= u:
            softmax_stage(n_soft)
            n_soft += 1
        pt, l1 = tiles.pop((u, half))
        c0 = half * H2 + j * 128
        vg = pltpu.bitcast(vv_ref[sl, :, c0:c0 + 128], bf16)
        acc = jnp.dot(vg, pt, preferred_element_type=f32)
        if ti in accs:
            prev = accs[ti]
            if ties and ties[0][0] <= len(hist):
                prev = jnp.concatenate(
                    [prev[0:24], jnp.where(never, ties.pop(0)[1], prev[24:32])], axis=0)
            acc = prev + acc
        accs[ti], nacc[ti] = acc, nacc.get(ti, 0) + 1
        if nacc[ti] == 2 * UT:
            assert ti == n_out
            l = jnp.sum(functools.reduce(jnp.add, lsum[ti]), axis=0, keepdims=True)
            o_ref[h0 + a, :, i * TQ:(i + 1) * TQ] = (acc * (1.0 / l)).astype(o_ref.dtype)
            n_out += 1
            for fn in events.pop(n_out, []):
                fn()
        for it in sched.pop(len(hist), []):
            it()
        hist.append(l1)
    assert not sched and not ties and not events


def _exact_head(h, refs):
    q_ref, k_ref, v_ref, o_ref = refs[:4]
    D, S = v_ref.shape[1], v_ref.shape[2]

    def body(it, carry):
        cols = pl.ds(pl.multiple_of(it * _TS, _TS), _TS)
        s = lax.dot_general(k_ref[h], q_ref[h, :, cols], (((0,), (0,)), ((), ())),
                            preferred_element_type=f32)
        p = jnp.exp2((s - jnp.max(s, axis=0, keepdims=True)) * _scale(D))
        l = jnp.sum(p, axis=0, keepdims=True)
        acc = jnp.dot(v_ref[h], p.astype(bf16), preferred_element_type=f32)
        o_ref[h, :, cols] = (acc * (1.0 / l)).astype(o_ref.dtype)
        return carry

    lax.fori_loop(0, S // _TS, body, 0)


def _kernel(q_hbm, k_hbm, v_hbm, o_hbm, in_ref, o_ref,
            kk_ref, vv_ref, mm_ref, safe_ref, probe_ref, sem_in, sem_out):
    HPS = _HPS
    n_heads, _, S = o_ref.shape
    n_tiles = S // _TQ
    n_blocks = (n_heads - 1) // HPS
    refs = (in_ref.at[1], in_ref.at[0], in_ref.at[2], o_ref,
            kk_ref, vv_ref, mm_ref, safe_ref)
    part = functools.partial

    def start_in(h, n, s):
        for a, hbm in enumerate((k_hbm, q_hbm, v_hbm)):
            pltpu.make_async_copy(hbm.at[pl.ds(h, n)], in_ref.at[a, pl.ds(h, n)],
                                  sem_in.at[s]).start()

    def wait_in(h, n, s):
        dst = in_ref.at[:, pl.ds(h, n)]
        pltpu.make_async_copy(dst, dst, sem_in.at[s]).wait()

    edges = [min(e, n_heads) for e in (2, 2 + HPS, 2 + 2 * HPS, n_heads)]
    sets = [(edges[i], edges[i + 1] - edges[i], 2 + i) for i in range(3)
            if edges[i + 1] > edges[i]]

    def copy_out(h, n, t0, t1):
        cols = pl.ds(t0 * _TQ, (t1 - t0) * _TQ)
        return pltpu.make_async_copy(o_ref.at[pl.ds(h, n), :, cols],
                                     o_hbm.at[pl.ds(h, n), :, cols], sem_out.at[0])

    def run_block(h0, slots, events):
        last = len(slots) - 1
        outs = [(last * n_tiles + 1, h0, last, 0, n_tiles),
                (last * n_tiles + _OSPLIT, h0 + last, 1, 0, _OSPLIT),
                ((last + 1) * n_tiles, h0 + last, 1, _OSPLIT, n_tiles)]
        for at, *args in outs[0 if last else 1:]:
            events.setdefault(at, []).append(lambda args=args: copy_out(*args).start())
        _packed_heads(h0, slots, refs, probe_ref[0] > 1e30, events)

    start_in(0, 1, 0)
    start_in(1, 1, 1)
    probe = _accumulation_probe()
    probe_ref[0] = probe[0]
    probe_ref[1] = jnp.min(jnp.where(probe == 0.5625, 1.0, 0.0), axis=0)
    wait_in(0, 1, 0)
    _prep_head(0, HPS - 1, refs)
    wait_in(1, 1, 1)
    run_block(0, [HPS - 1], {0: [part(start_in, *sets[0])],
                             n_tiles - 1: [part(start_in, *st) for st in sets[1:]]})

    def block(b, carry):
        for i, st in enumerate(sets):
            pl.when(b == i)(part(wait_in, *st))
        run_block(1 + b * HPS, list(range(HPS)), {})
        return carry

    lax.fori_loop(0, n_blocks, block, 0)

    all_safe = jnp.min(jnp.minimum(jnp.min(safe_ref[...], axis=0), probe_ref[1]))
    pltpu.make_async_copy(o_ref, o_hbm, sem_out.at[0]).wait()

    @pl.when(all_safe < 0.5)
    def _():
        def fix(h, carry):
            @pl.when(jnp.min(jnp.minimum(safe_ref[h], probe_ref[1])) < 0.5)
            def _():
                _exact_head(h, refs)
                cp = copy_out(h, 1, 0, n_tiles)
                cp.start()
                cp.wait()
            return carry

        lax.fori_loop(0, n_heads, fix, 0)


@jax.jit
def pallas_standalone__fused_io_aware_attn__prompt_kernel(
    q: jax.Array,
    k: jax.Array,
    v: jax.Array,
):
    B, H, S, D = q.shape
    n_heads = B * H
    assert D == 32 and S % 512 == 0 and (n_heads - 1) % _HPS == 0
    qt, kt, vt = (jnp.swapaxes(x, -1, -2).reshape(n_heads, D, S) for x in (q, k, v))
    hbm = pl.BlockSpec(memory_space=pl.ANY)
    ot = pl.pallas_call(
        _kernel,
        in_specs=[hbm] * 3,
        out_specs=hbm,
        out_shape=jax.ShapeDtypeStruct((n_heads, D, S), q.dtype),
        scratch_shapes=[
            pltpu.VMEM((3, n_heads, D, S), q.dtype),
            pltpu.VMEM((n_heads, D, S), q.dtype),
            pltpu.VMEM((_HPS, S // 4, 128), u32),
            pltpu.VMEM((_HPS, D // 2, S), u32),
            pltpu.VMEM((_HPS, 2, 8, 128), f32),
            pltpu.VMEM((n_heads, 8, 128), f32),
            pltpu.VMEM((2, 8, 128), f32),
            pltpu.SemaphoreType.DMA((5,)),
            pltpu.SemaphoreType.DMA((1,)),
        ],
        compiler_params=pltpu.CompilerParams(
            vmem_limit_bytes=96 << 20,
            disable_bounds_checks=True),
    )(qt, kt, vt)
    return jnp.swapaxes(ot.reshape(B, H, D, S), -1, -2)
```

```python
import functools
import math

import jax
import jax.numpy as jnp
from jax import lax
import jax.experimental.pallas as pl
import jax.experimental.pallas.tpu as pltpu

f32, bf16, u32, i32 = jnp.float32, jnp.bfloat16, jnp.uint32, jnp.int32

_TQ = 128
_KD = 80
_ORDER = (6, 4, 2, 0, 7, 5, 3, 1)
_T_MAX = 64.0
_HPS = 7
_NL = 4
_TS = 512
_FIRST = 3
_OSPLIT = 14
_PREFIX = ("QQ", "QQ", "QQPPP", "QQPPP")
_TAILP = 6
_P0, _PEND, _GAP, _AFT, _TDLY = 16, 32, 3, 3, 4


def _scale(d):
    return (d ** -0.5) * math.log2(math.e)


def _sumsq(x):
    y = x * x
    return (y[0:8] + y[8:16]) + (y[16:24] + y[24:32])


def _prep_items(h, slot, refs, tie, after):
    q_ref, k_ref, v_ref, _, kk_ref, vv_ref, mm_ref, safe_ref = refs
    D, S = q_ref.shape[1], q_ref.shape[2]
    H2 = S // 2
    c = _scale(D)
    st = {}

    def norm_item(key, ref, i):
        n2 = after(_sumsq(ref[h, :, i * 128:(i + 1) * 128].astype(f32)))
        st[key] = jnp.maximum(st[key], n2) if key in st else n2
        tie(st[key])

    def bound_item():
        def top(x):
            x = jnp.sum(x, axis=0, keepdims=True)
            return jnp.max(x, axis=1, keepdims=True) + 2.0 ** -120
        b2 = jnp.broadcast_to(top(st['q']) * top(st['k']) * (1.04 * c * c), (8, 128))
        safe_ref[h] = jnp.where(b2 < _T_MAX * _T_MAX, 1.0, 0.0)
        b2 = jnp.minimum(jnp.maximum(b2, 2.0 ** -40), _T_MAX * _T_MAX)
        e = (pltpu.bitcast(b2, i32) >> 23) - 127
        p2 = pltpu.bitcast(((e >> 1) + 128) << 23, f32)
        cm = p2 * 3072.0
        row = lax.broadcasted_iota(i32, (8, 128), 0)
        cz = jnp.where(row == 0, cm, jnp.where(row == 4, -cm, 0.0))
        crow = pltpu.bitcast(pltpu.bitcast(cz, u32) >> 16, f32)
        mm_ref[slot, 0] = cm
        mm_ref[slot, 1] = crow
        tie(crow)

    def k_item(t):
        ka = k_ref[h, :, t * 128:(t + 1) * 128].astype(f32)
        kb = k_ref[h, :, H2 + t * 128:H2 + (t + 1) * 128].astype(f32)
        xt = jnp.concatenate(
            [ka * c, jnp.ones((16, 128), f32), kb * (c * 2.0 ** -13),
             jnp.zeros((48, 128), f32)], axis=0).astype(bf16)
        kt = pltpu.bitcast(xt.T, u32)
        kk_ref[slot, t * 64:(t + 1) * 64, :] = jnp.concatenate(
            [kt[8 * w:8 * w + 8] for w in _ORDER], axis=0)
        tie(pltpu.bitcast(kt[56:64], f32))

    def v_item(t):
        lane = lax.broadcasted_iota(i32, (16, 128), 1)
        sel = (lane & 16) == 0
        def load(c0):
            x = pltpu.bitcast(v_ref[h, :, c0:c0 + 128], f32)
            x = jnp.concatenate([after(x[0:8]), after(x[8:16])], axis=0)
            return pltpu.bitcast(x, u32)
        va, vb = load(t * 128), load(H2 + t * 128)
        v1 = jnp.where(sel, va, pltpu.roll(vb, 16, 1))
        v2 = jnp.where(sel, pltpu.roll(va, 112, 1), vb)
        vv_ref[slot, :, t * 128:(t + 1) * 128] = v1
        vv_ref[slot, :, H2 + t * 128:H2 + (t + 1) * 128] = v2
        for z in (v2[8:16], v2[0:8], v1[8:16], v1[0:8]):
            tie(pltpu.bitcast(z, f32))

    part = functools.partial
    gap = [None] * _GAP
    items = []
    for i in range(S // 128):
        items += [part(norm_item, 'q', q_ref, i), part(norm_item, 'k', k_ref, i)]
    items += gap + [bound_item] + gap
    for t in range(0, S // 256, 2):
        items += [part(k_item, t), part(k_item, t + 1)] + gap
    for t in range(S // 256):
        items += [part(v_item, t), None]
    return items


def _accumulation_probe():
    row = lax.broadcasted_iota(i32, (_KD, 128), 0)
    w = jnp.where(row < 32, 0.0107421875,
                  jnp.where(row == 32, 6291456.0,
                            jnp.where(row == 40, -6291456.0,
                                      jnp.where(row >= 48, 2.0 ** -9, 0.0))))
    return jnp.dot(jnp.ones((128, _KD), bf16), w.astype(bf16),
                   preferred_element_type=f32).reshape(16, 8, 128)


def _mxu_order(nu):
    qs, ps = [], []
    for m, pre in enumerate(_PREFIX):
        nq, npv = nu // 4 - pre.count('Q'), nu // 2 - pre.count('P')
        short = max(0, _TAILP - (npv - 2 * (nq - 1)))
        seq = pre + 'QPP' * (nq - 1 - short) + 'QP' * short + 'Q'
        seq += 'P' * (nu // 2 - seq.count('P'))
        tm = 0
        for ch in seq:
            (qs if ch == 'Q' else ps).append((tm, m))
            tm += 128 if ch == 'Q' else 32
    qs.sort()
    ps.sort()
    ops = {pos: ('Q', u, 0) for u, pos in enumerate(qs)}
    ready = sorted((tm + 64 * (half + 1), u, half)
                   for u, (tm, _) in enumerate(qs) for half in range(2))
    for pos, (_, u, half) in zip(ps, ready):
        ops[pos] = ('P', u, half)
    return [ops[pos] for pos in sorted(ops)]


def _packed_heads(h0, slots, refs, never, events, t0=0, t1=None, prep=True):
    q_ref, _, v_ref, o_ref, kk_ref, vv_ref, mm_ref, _ = refs
    S = v_ref.shape[2]
    H2 = S // 2
    TQ = _TQ
    UT = H2 // 128
    t1 = S // TQ if t1 is None else t1
    UH = (t1 - t0) * UT
    PH = 2 * UH
    xs, tiles, ties, sched, hist = {}, {}, [], {}, []
    qws, cms, lsum, accs, nacc = {}, {}, {}, {}, {}

    def tie(v):
        ties.append((len(hist) + _TDLY, v))

    def after(x):
        return jnp.where(never, hist[-_AFT], x)

    for a in range(len(slots) if prep else 0):
        if a + 1 < len(slots):
            hn, sn = h0 + a + 1, slots[a + 1]
        else:
            hn, sn = jnp.minimum(h0 + a + 1, q_ref.shape[0] - 1), 0
        items = _prep_items(hn, sn, refs, tie, after)
        for b, it in enumerate(items):
            if it is not None:
                at = a * PH + _P0 + b * (PH - _P0 - _PEND) // len(items)
                sched.setdefault(at, []).append(it)

    def softmax_stage(u):
        cm = cms[u // UH]
        l_run = lsum.setdefault(u // UT, [None] * _NL)
        lg = u % _NL
        x = xs.pop(u).reshape(8, 2, 8, 128)
        hi = (x + cm) - cm
        ph = jnp.exp2(hi)
        plo = jnp.exp2((x - hi) * 8192.0)
        ps = jnp.sum((ph + plo).reshape(2, 8, 8, 128), axis=1)
        p = jnp.concatenate([ph, plo], axis=1).reshape(256, 128)
        for half in range(2):
            s1 = ps[half]
            l1 = l_run[lg] = s1 if l_run[lg] is None else l_run[lg] + s1
            r = half * 128
            pt = jnp.concatenate(
                [jnp.where(never, l1, p[r + 96:r + 104]), p[r + 104:r + 128],
                 p[r + 64:r + 96], p[r + 32:r + 64], p[r:r + 32]], axis=0)
            tiles[(u, half)] = (pt.astype(bf16), l1)

    n_soft = n_out = 0
    for kind, u, half in _mxu_order(UH * len(slots)):
        a, rem = divmod(u, UH)
        i, j = divmod(rem, UT)
        i += t0
        sl = slots[a]
        ti = u // UT
        if kind == 'Q':
            if u // 2 not in qws:
                qu = pltpu.bitcast(q_ref[h0 + a, :, i * TQ:(i + 1) * TQ], u32)
                qws[u // 2] = pltpu.bitcast(jnp.concatenate(
                    [qu, pltpu.bitcast(mm_ref[sl, 1], u32), qu], axis=0), bf16)
            kg = pltpu.bitcast(kk_ref[sl, j * 64:(j + 1) * 64, :], bf16)[:, :_KD]
            xs[u] = jnp.dot(kg, qws[u // 2], preferred_element_type=f32)
            if a not in cms:
                cms[a] = mm_ref[sl, 0][None, None]
            continue
        while n_soft <= u:
            softmax_stage(n_soft)
            n_soft += 1
        pt, l1 = tiles.pop((u, half))
        c0 = half * H2 + j * 128
        vg = pltpu.bitcast(vv_ref[sl, :, c0:c0 + 128], bf16)
        acc = jnp.dot(vg, pt, preferred_element_type=f32)
        if ti in accs:
            prev = accs[ti]
            if ties and ties[0][0] <= len(hist):
                prev = jnp.concatenate(
                    [prev[0:24], jnp.where(never, ties.pop(0)[1], prev[24:32])], axis=0)
            acc = prev + acc
        accs[ti], nacc[ti] = acc, nacc.get(ti, 0) + 1
        if nacc[ti] == 2 * UT:
            assert ti == n_out
            l = jnp.sum(functools.reduce(jnp.add, lsum[ti]), axis=0, keepdims=True)
            o_ref[h0 + a, :, i * TQ:(i + 1) * TQ] = (acc * (1.0 / l)).astype(o_ref.dtype)
            n_out += 1
            for fn in events.pop(n_out, []):
                fn()
        for it in sched.pop(len(hist), []):
            it()
        hist.append(l1)
    assert not sched and not ties and not events


def _exact_head(h, refs):
    q_ref, k_ref, v_ref, o_ref = refs[:4]
    D, S = v_ref.shape[1], v_ref.shape[2]

    def body(it, carry):
        cols = pl.ds(pl.multiple_of(it * _TS, _TS), _TS)
        s = lax.dot_general(k_ref[h], q_ref[h, :, cols], (((0,), (0,)), ((), ())),
                            preferred_element_type=f32)
        s = (s.astype(bf16) * D ** -0.5).astype(f32)
        p = jnp.exp(s - jnp.max(s, axis=0, keepdims=True))
        l = jnp.sum(p, axis=0, keepdims=True)
        acc = jnp.dot(v_ref[h], p.astype(bf16), preferred_element_type=f32)
        o_ref[h, :, cols] = (acc * (1.0 / l)).astype(o_ref.dtype)
        return carry

    lax.fori_loop(0, S // _TS, body, 0)


def _kernel(q_hbm, k_hbm, v_hbm, o_hbm, in_ref, o_ref,
            kk_ref, vv_ref, mm_ref, safe_ref, probe_ref, sem_in, sem_out):
    HPS = _HPS
    n_heads, _, S = o_ref.shape
    n_tiles = S // _TQ
    n_blocks = (n_heads - 1) // HPS
    refs = (in_ref.at[1], in_ref.at[0], in_ref.at[2], o_ref,
            kk_ref, vv_ref, mm_ref, safe_ref)
    part = functools.partial

    def start_in(h, n, s, a0=0, a1=3):
        for a in range(a0, a1):
            hbm = (k_hbm, q_hbm, v_hbm)[a]
            pltpu.make_async_copy(hbm.at[pl.ds(h, n)], in_ref.at[a, pl.ds(h, n)],
                                  sem_in.at[s]).start()

    def wait_in(h, n, s, a0=0, a1=3):
        dst = in_ref.at[pl.ds(a0, a1 - a0), pl.ds(h, n)]
        pltpu.make_async_copy(dst, dst, sem_in.at[s]).wait()

    edges = [min(e, n_heads) for e in (2, 2 + HPS, 2 + 2 * HPS, n_heads)]
    sets = [(edges[i], edges[i + 1] - edges[i], 2 + i) for i in range(3)
            if edges[i + 1] > edges[i]]

    def copy_out(h, n, t0, t1):
        cols = pl.ds(t0 * _TQ, (t1 - t0) * _TQ)
        return pltpu.make_async_copy(o_ref.at[pl.ds(h, n), :, cols],
                                     o_hbm.at[pl.ds(h, n), :, cols], sem_out.at[0])

    def run_block(h0, slots, t0=0):
        last = len(slots) - 1
        outs = [(last * n_tiles + 1, h0, last, 0, n_tiles),
                (last * n_tiles + _OSPLIT - t0, h0 + last, 1, 0, _OSPLIT),
                ((last + 1) * n_tiles - t0, h0 + last, 1, _OSPLIT, n_tiles)]
        events = {at: [lambda args=args: copy_out(*args).start()]
                  for at, *args in outs[0 if last else 1:]}
        _packed_heads(h0, slots, refs, probe_ref[0] > 1e30, events, t0=t0)

    start_in(0, 1, 0, 0, 2)
    start_in(0, 1, 5, 2, 3)
    start_in(1, 1, 1)
    for st in sets:
        start_in(*st)
    probe = _accumulation_probe()
    probe_ref[0] = probe[0]
    probe_ref[1] = jnp.min(jnp.where(probe == 0.5625, 1.0, 0.0), axis=0)
    items = [it for it in _prep_items(0, HPS - 1, refs, lambda x: None, lambda x: x)
             if it is not None]
    n_v = S // 256 + 4
    wait_in(0, 1, 0, 0, 2)
    for it in items[:-n_v]:
        it()
    wait_in(0, 1, 5, 2, 3)
    for it in items[-n_v:]:
        it()
    _packed_heads(0, [HPS - 1], refs, probe_ref[0] > 1e30, {}, t1=_FIRST, prep=False)
    wait_in(1, 1, 1)
    run_block(0, [HPS - 1], _FIRST)

    def block(b, carry):
        for i, st in enumerate(sets):
            pl.when(b == i)(part(wait_in, *st))
        run_block(1 + b * HPS, list(range(HPS)))
        return carry

    lax.fori_loop(0, n_blocks, block, 0)

    all_safe = jnp.min(jnp.minimum(jnp.min(safe_ref[...], axis=0), probe_ref[1]))
    pltpu.make_async_copy(o_ref, o_hbm, sem_out.at[0]).wait()

    @pl.when(all_safe < 0.5)
    def _():
        def fix(h, carry):
            @pl.when(jnp.min(jnp.minimum(safe_ref[h], probe_ref[1])) < 0.5)
            def _():
                _exact_head(h, refs)
                cp = copy_out(h, 1, 0, n_tiles)
                cp.start()
                cp.wait()
            return carry

        lax.fori_loop(0, n_heads, fix, 0)


@jax.jit
def pallas_standalone__fused_io_aware_attn__prompt_kernel(
    q: jax.Array,
    k: jax.Array,
    v: jax.Array,
):
    B, H, S, D = q.shape
    n_heads = B * H
    assert D == 32 and S % 512 == 0 and (n_heads - 1) % _HPS == 0
    qt, kt, vt = (jnp.swapaxes(x, -1, -2).reshape(n_heads, D, S) for x in (q, k, v))
    hbm = pl.BlockSpec(memory_space=pl.ANY)
    ot = pl.pallas_call(
        _kernel,
        in_specs=[hbm] * 3,
        out_specs=hbm,
        out_shape=jax.ShapeDtypeStruct((n_heads, D, S), q.dtype),
        scratch_shapes=[
            pltpu.VMEM((3, n_heads, D, S), q.dtype),
            pltpu.VMEM((n_heads, D, S), q.dtype),
            pltpu.VMEM((_HPS, S // 4, 128), u32),
            pltpu.VMEM((_HPS, D // 2, S), u32),
            pltpu.VMEM((_HPS, 2, 8, 128), f32),
            pltpu.VMEM((n_heads, 8, 128), f32),
            pltpu.VMEM((2, 8, 128), f32),
            pltpu.SemaphoreType.DMA((6,)),
            pltpu.SemaphoreType.DMA((1,)),
        ],
        compiler_params=pltpu.CompilerParams(
            vmem_limit_bytes=96 << 20,
            disable_bounds_checks=True),
    )(qt, kt, vt)
    return jnp.swapaxes(ot.reshape(B, H, D, S), -1, -2)
```

```python
import functools
import math

import jax
import jax.numpy as jnp
from jax import lax
import jax.experimental.pallas as pl
import jax.experimental.pallas.tpu as pltpu

f32, bf16, u32, i32 = jnp.float32, jnp.bfloat16, jnp.uint32, jnp.int32

_TQ = 128
_KD = 80
_ORDER = (6, 4, 2, 0, 7, 5, 3, 1)
_T_MAX = 64.0
_HPS = 7
_NL = 4
_TS = 512
_FIRST = 3
_OSPLIT = 14
_PREFIX = ("QQ", "QQ", "QQPPP", "QQPPP")
_TAILP = 6
_P0, _PEND, _GAP, _AFT, _TDLY = 16, 32, 3, 3, 4


def _scale(d):
    return (d ** -0.5) * math.log2(math.e)


def _sumsq(x):
    y = x * x
    return (y[0:8] + y[8:16]) + (y[16:24] + y[24:32])


def _prep_items(h, slot, refs, tie, after):
    q_ref, k_ref, v_ref, _, kk_ref, vv_ref, mm_ref, safe_ref = refs
    D, S = q_ref.shape[1], q_ref.shape[2]
    H2 = S // 2
    c = _scale(D)
    st = {}

    def norm_item(key, ref, i):
        n2 = after(_sumsq(ref[h, :, i * 128:(i + 1) * 128].astype(f32)))
        st[key] = jnp.maximum(st[key], n2) if key in st else n2
        tie(st[key])

    def bound_item():
        def top(x):
            x = jnp.sum(x, axis=0, keepdims=True)
            return jnp.max(x, axis=1, keepdims=True) + 2.0 ** -120
        b2 = jnp.broadcast_to(top(st['q']) * top(st['k']) * (1.04 * c * c), (8, 128))
        safe_ref[h] = jnp.where(b2 < _T_MAX * _T_MAX, 1.0, 0.0)
        b2 = jnp.minimum(jnp.maximum(b2, 2.0 ** -40), _T_MAX * _T_MAX)
        e = (pltpu.bitcast(b2, i32) >> 23) - 127
        p2 = pltpu.bitcast(((e >> 1) + 128) << 23, f32)
        cm = p2 * 3072.0
        row = lax.broadcasted_iota(i32, (8, 128), 0)
        cz = jnp.where(row == 0, cm, jnp.where(row == 4, -cm, 0.0))
        crow = pltpu.bitcast(cz, u32) >> 16
        mm_ref[slot, 0] = pltpu.bitcast(cm, u32)
        mm_ref[slot, 1] = crow
        tie(crow)

    def k_item(t):
        ka = k_ref[h, :, t * 128:(t + 1) * 128].astype(f32)
        kb = k_ref[h, :, H2 + t * 128:H2 + (t + 1) * 128].astype(f32)
        xt = jnp.concatenate(
            [ka * c, jnp.ones((16, 128), f32), kb * (c * 2.0 ** -13),
             jnp.zeros((48, 128), f32)], axis=0).astype(bf16)
        kt = pltpu.bitcast(xt.T, u32)
        kk_ref[slot, t * 64:(t + 1) * 64, :] = jnp.concatenate(
            [kt[8 * w:8 * w + 8] for w in _ORDER], axis=0)
        tie(kt[56:64])

    def v_item(t):
        lane = lax.broadcasted_iota(i32, (16, 128), 1)
        sel = (lane & 16) == 0

        def load(c0):
            x = pltpu.bitcast(v_ref[h, :, c0:c0 + 128], u32)
            return jnp.concatenate([after(x[0:8]), after(x[8:16])], axis=0)

        va, vb = load(t * 128), load(H2 + t * 128)
        v1 = jnp.where(sel, va, pltpu.roll(vb, 16, 1))
        v2 = jnp.where(sel, pltpu.roll(va, 112, 1), vb)
        vv_ref[slot, :, t * 128:(t + 1) * 128] = v1
        vv_ref[slot, :, H2 + t * 128:H2 + (t + 1) * 128] = v2
        for z in (v2[8:16], v2[0:8], v1[8:16], v1[0:8]):
            tie(z)

    part = functools.partial
    gap = [None] * _GAP
    items = []
    for i in range(S // 128):
        items += [part(norm_item, 'q', q_ref, i), part(norm_item, 'k', k_ref, i)]
    items += gap + [bound_item] + gap
    for t in range(0, S // 256, 2):
        items += [part(k_item, t), part(k_item, t + 1)] + gap
    for t in range(S // 256):
        items += [part(v_item, t), None]
    return items


def _accumulation_probe():
    row = lax.broadcasted_iota(i32, (_KD, 128), 0)
    w = jnp.where(row < 32, 0.0107421875,
                  jnp.where(row == 32, 6291456.0,
                            jnp.where(row == 40, -6291456.0,
                                      jnp.where(row >= 48, 2.0 ** -9, 0.0))))
    return jnp.dot(jnp.ones((128, _KD), bf16), w.astype(bf16),
                   preferred_element_type=f32).reshape(16, 8, 128)


def _mxu_order(nu):
    qs, ps = [], []
    for m, pre in enumerate(_PREFIX):
        nq, npv = nu // 4 - pre.count('Q'), nu // 2 - pre.count('P')
        short = max(0, _TAILP - (npv - 2 * (nq - 1)))
        seq = pre + 'QPP' * (nq - 1 - short) + 'QP' * short + 'Q'
        seq += 'P' * (nu // 2 - seq.count('P'))
        tm = 0
        for ch in seq:
            (qs if ch == 'Q' else ps).append((tm, m))
            tm += 128 if ch == 'Q' else 32
    qs.sort()
    ps.sort()
    ops = {pos: ('Q', u, 0) for u, pos in enumerate(qs)}
    ready = sorted((tm + 64 * (half + 1), u, half)
                   for u, (tm, _) in enumerate(qs) for half in range(2))
    for pos, (_, u, half) in zip(ps, ready):
        ops[pos] = ('P', u, half)
    return [ops[pos] for pos in sorted(ops)]


def _packed_heads(h0, slots, refs, never, events, t0=0, t1=None, prep=True):
    q_ref, _, v_ref, o_ref, kk_ref, vv_ref, mm_ref, _ = refs
    S = v_ref.shape[2]
    H2 = S // 2
    TQ = _TQ
    UT = H2 // 128
    t1 = S // TQ if t1 is None else t1
    UH = (t1 - t0) * UT
    PH = 2 * UH
    xs, tiles, ties, sched, hist = {}, {}, [], {}, []
    qws, cms, lsum, accs, nacc = {}, {}, {}, {}, {}

    def pin(v, x):
        if v.dtype != x.dtype:
            v = pltpu.bitcast(v, x.dtype)
        return jnp.where(never, v, x)

    def tie(v):
        ties.append((len(hist) + _TDLY, v))

    def after(x):
        return pin(hist[-_AFT], x)

    for a in range(len(slots) if prep else 0):
        if a + 1 < len(slots):
            hn, sn = h0 + a + 1, slots[a + 1]
        else:
            hn, sn = jnp.minimum(h0 + a + 1, q_ref.shape[0] - 1), 0
        items = _prep_items(hn, sn, refs, tie, after)
        for b, it in enumerate(items):
            if it is not None:
                at = a * PH + _P0 + b * (PH - _P0 - _PEND) // len(items)
                sched.setdefault(at, []).append(it)

    def softmax_stage(u):
        cm = cms[u // UH]
        l_run = lsum.setdefault(u // UT, [None] * _NL)
        lg = u % _NL
        x = xs.pop(u).reshape(8, 2, 8, 128)
        hi = (x + cm) - cm
        ph = jnp.exp2(hi)
        plo = jnp.exp2((x - hi) * 8192.0)
        ps = jnp.sum((ph + plo).reshape(2, 8, 8, 128), axis=1)
        p = jnp.concatenate([ph, plo], axis=1).reshape(256, 128)
        for half in range(2):
            s1 = ps[half]
            l1 = l_run[lg] = s1 if l_run[lg] is None else l_run[lg] + s1
            r = half * 128
            pt = jnp.concatenate(
                [pin(l1, p[r + 96:r + 104]), p[r + 104:r + 128],
                 p[r + 64:r + 96], p[r + 32:r + 64], p[r:r + 32]], axis=0)
            tiles[(u, half)] = (pt.astype(bf16), l1)

    n_soft = n_out = 0
    for kind, u, half in _mxu_order(UH * len(slots)):
        a, rem = divmod(u, UH)
        i, j = divmod(rem, UT)
        i += t0
        sl = slots[a]
        ti = u // UT
        if kind == 'Q':
            if u // 2 not in qws:
                qu = pltpu.bitcast(q_ref[h0 + a, :, i * TQ:(i + 1) * TQ], u32)
                qws[u // 2] = pltpu.bitcast(jnp.concatenate(
                    [qu, mm_ref[sl, 1], qu], axis=0), bf16)
            kg = pltpu.bitcast(kk_ref[sl, j * 64:(j + 1) * 64, :], bf16)[:, :_KD]
            xs[u] = jnp.dot(kg, qws[u // 2], preferred_element_type=f32)
            if a not in cms:
                assert all(at >= a * PH for at in sched)
                cms[a] = pltpu.bitcast(mm_ref[sl, 0], f32)[None, None]
            continue
        while n_soft <= u:
            softmax_stage(n_soft)
            n_soft += 1
        pt, l1 = tiles.pop((u, half))
        c0 = half * H2 + j * 128
        vg = pltpu.bitcast(vv_ref[sl, :, c0:c0 + 128], bf16)
        acc = jnp.dot(vg, pt, preferred_element_type=f32)
        if ti in accs:
            prev = accs[ti]
            if ties and ties[0][0] <= len(hist):
                prev = jnp.concatenate(
                    [prev[0:24], pin(ties.pop(0)[1], prev[24:32])], axis=0)
            acc = prev + acc
        accs[ti], nacc[ti] = acc, nacc.get(ti, 0) + 1
        if nacc[ti] == 2 * UT:
            assert ti == n_out
            l = jnp.sum(functools.reduce(jnp.add, lsum[ti]), axis=0, keepdims=True)
            o_ref[h0 + a, :, i * TQ:(i + 1) * TQ] = (acc * (1.0 / l)).astype(o_ref.dtype)
            n_out += 1
            for fn in events.pop(n_out, []):
                fn()
        for it in sched.pop(len(hist), []):
            it()
        hist.append(l1)
    assert not sched and not ties and not events


def _exact_head(h, refs):
    q_ref, k_ref, v_ref, o_ref = refs[:4]
    D, S = v_ref.shape[1], v_ref.shape[2]

    def body(it, carry):
        cols = pl.ds(pl.multiple_of(it * _TS, _TS), _TS)
        s = lax.dot_general(k_ref[h], q_ref[h, :, cols], (((0,), (0,)), ((), ())),
                            preferred_element_type=f32)
        s = (s.astype(bf16) * D ** -0.5).astype(f32)
        p = jnp.exp(s - jnp.max(s, axis=0, keepdims=True))
        l = jnp.sum(p, axis=0, keepdims=True)
        acc = jnp.dot(v_ref[h], p.astype(bf16), preferred_element_type=f32)
        o_ref[h, :, cols] = (acc * (1.0 / l)).astype(o_ref.dtype)
        return carry

    lax.fori_loop(0, S // _TS, body, 0)


def _kernel(q_hbm, k_hbm, v_hbm, o_hbm, in_ref, o_ref,
            kk_ref, vv_ref, mm_ref, safe_ref, probe_ref, sem_in, sem_out):
    HPS = _HPS
    n_heads, _, S = o_ref.shape
    n_tiles = S // _TQ
    n_blocks = (n_heads - 1) // HPS
    refs = (in_ref.at[1], in_ref.at[0], in_ref.at[2], o_ref,
            kk_ref, vv_ref, mm_ref, safe_ref)
    part = functools.partial

    def start_in(h, n, s, a0=0, a1=3):
        for a in range(a0, a1):
            hbm = (k_hbm, q_hbm, v_hbm)[a]
            pltpu.make_async_copy(hbm.at[pl.ds(h, n)], in_ref.at[a, pl.ds(h, n)],
                                  sem_in.at[s]).start()

    def wait_in(h, n, s, a0=0, a1=3):
        dst = in_ref.at[pl.ds(a0, a1 - a0), pl.ds(h, n)]
        pltpu.make_async_copy(dst, dst, sem_in.at[s]).wait()

    edges = [min(e, n_heads) for e in (2, 2 + HPS, 2 + 2 * HPS, n_heads)]
    sets = [(edges[i], edges[i + 1] - edges[i], 2 + i) for i in range(3)
            if edges[i + 1] > edges[i]]

    def copy_out(h, n, t0, t1):
        cols = pl.ds(t0 * _TQ, (t1 - t0) * _TQ)
        return pltpu.make_async_copy(o_ref.at[pl.ds(h, n), :, cols],
                                     o_hbm.at[pl.ds(h, n), :, cols], sem_out.at[0])

    def run_block(h0, slots, t0=0):
        last = len(slots) - 1
        outs = [(last * n_tiles + 1, h0, last, 0, n_tiles),
                (last * n_tiles + _OSPLIT - t0, h0 + last, 1, 0, _OSPLIT),
                ((last + 1) * n_tiles - t0, h0 + last, 1, _OSPLIT, n_tiles)]
        events = {at: [lambda args=args: copy_out(*args).start()]
                  for at, *args in outs[0 if last else 1:]}
        _packed_heads(h0, slots, refs, probe_ref[0] > 1e30, events, t0=t0)

    start_in(0, 1, 0, 0, 2)
    start_in(0, 1, 5, 2, 3)
    start_in(1, 1, 1)
    for st in sets:
        start_in(*st)
    probe = _accumulation_probe()
    probe_ref[0] = probe[0]
    probe_ref[1] = jnp.min(jnp.where(probe == 0.5625, 1.0, 0.0), axis=0)
    items = [it for it in _prep_items(0, HPS - 1, refs, lambda x: None, lambda x: x)
             if it is not None]
    n_v = S // 256 + 4
    wait_in(0, 1, 0, 0, 2)
    for it in items[:-n_v]:
        it()
    wait_in(0, 1, 5, 2, 3)
    for it in items[-n_v:]:
        it()
    _packed_heads(0, [HPS - 1], refs, probe_ref[0] > 1e30, {}, t1=_FIRST, prep=False)
    wait_in(1, 1, 1)
    run_block(0, [HPS - 1], _FIRST)

    def block(b, carry):
        for i, st in enumerate(sets):
            pl.when(b == i)(part(wait_in, *st))
        run_block(1 + b * HPS, list(range(HPS)))
        return carry

    lax.fori_loop(0, n_blocks, block, 0)

    all_safe = jnp.min(jnp.minimum(jnp.min(safe_ref[...], axis=0), probe_ref[1]))
    pltpu.make_async_copy(o_ref, o_hbm, sem_out.at[0]).wait()

    @pl.when(all_safe < 0.5)
    def _():
        def fix(h, carry):
            @pl.when(jnp.min(jnp.minimum(safe_ref[h], probe_ref[1])) < 0.5)
            def _():
                _exact_head(h, refs)
                cp = copy_out(h, 1, 0, n_tiles)
                cp.start()
                cp.wait()
            return carry

        lax.fori_loop(0, n_heads, fix, 0)


@jax.jit
def pallas_standalone__fused_io_aware_attn__prompt_kernel(
    q: jax.Array,
    k: jax.Array,
    v: jax.Array,
):
    B, H, S, D = q.shape
    n_heads = B * H
    assert D == 32 and S % 512 == 0 and (n_heads - 1) % _HPS == 0
    qt, kt, vt = (jnp.swapaxes(x, -1, -2).reshape(n_heads, D, S) for x in (q, k, v))
    hbm = pl.BlockSpec(memory_space=pl.ANY)
    ot = pl.pallas_call(
        _kernel,
        in_specs=[hbm] * 3,
        out_specs=hbm,
        out_shape=jax.ShapeDtypeStruct((n_heads, D, S), q.dtype),
        scratch_shapes=[
            pltpu.VMEM((3, n_heads, D, S), q.dtype),
            pltpu.VMEM((n_heads, D, S), q.dtype),
            pltpu.VMEM((_HPS, S // 4, 128), u32),
            pltpu.VMEM((_HPS, D // 2, S), u32),
            pltpu.VMEM((_HPS, 2, 8, 128), u32),
            pltpu.VMEM((n_heads, 8, 128), f32),
            pltpu.VMEM((2, 8, 128), f32),
            pltpu.SemaphoreType.DMA((6,)),
            pltpu.SemaphoreType.DMA((1,)),
        ],
        compiler_params=pltpu.CompilerParams(
            vmem_limit_bytes=96 << 20,
            disable_bounds_checks=True),
    )(qt, kt, vt)
    return jnp.swapaxes(ot.reshape(B, H, D, S), -1, -2)
```
